```python
import os as _os
_os.environ.setdefault("JAX_PLATFORMS", "cpu")
import jax
import jax.numpy as jnp

def _softmax(x, axis=-1):
    return jax.nn.softmax(x, axis=axis)
def _gelu(x):
    return jax.nn.gelu(x, approximate=True)
def _silu(x):
    return jax.nn.silu(x)
def _sigmoid(x):
    return jax.nn.sigmoid(x)
def _layernorm(x, axis=-1, eps=1e-5):
    m = jnp.mean(x, axis=axis, keepdims=True)
    v = jnp.var(x, axis=axis, keepdims=True)
    return (x - m) / jnp.sqrt(v + eps)
def _scatter_add(tgt, idx, src, axis=0):
    return tgt.at[idx].add(src)
def _segment_sum(src, seg, n):
    return jax.ops.segment_sum(src, seg, n)
class _Rng:
    def __init__(self, key):
        self._k = key
    def _next(self):
        self._k, sub = jax.random.split(self._k)
        return sub
    def normal(self, shape):
        return jax.random.normal(self._next(), shape, dtype=jnp.bfloat16)
    def randint(self, lo, hi, shape):
        return jax.random.randint(self._next(), shape, lo, hi, dtype=jnp.int32)
    def uniform(self, shape, lo=0.0, hi=1.0):
        return jax.random.uniform(self._next(), shape, jnp.bfloat16, lo, hi)
    def permutation(self, n):
        return jax.random.permutation(self._next(), n)


kernel_name = 'parallel_sum__grouped_kv_mqa__dense_activation_silu__prompt'

def setup_inputs():
    _rng = _Rng(jax.random.key(int.from_bytes(__import__("os").urandom(4), "little")))
    _w = (lambda a: (lambda t: t.astype(jnp.bfloat16) if jnp.issubdtype(t.dtype, jnp.floating) else t)(jnp.asarray(a)))
    def _A_setup():
        B, S, D, H = 1, 2048, 512, 32
        Dh = D // H
        return {
            "x": _w((lambda *s: _rng.normal(s) * 0.05)(B, S, D)),
            "wq": _w((lambda *s: _rng.normal(s) * 0.05)(D, H * Dh)),
            "wk": _w((lambda *s: _rng.normal(s) * 0.05)(D, Dh)),
            "wv": _w((lambda *s: _rng.normal(s) * 0.05)(D, Dh)),
            "wo": _w((lambda *s: _rng.normal(s) * 0.05)(H * Dh, D)),
        }
    _A_in = _A_setup()

    def _B_setup():
        B, S, D, F = 1, 2048, 512, 1792
        return {
            "x": _w((lambda *s: _rng.normal(s) * 0.05)(B, S, D)),
            "w1": _w((lambda *s: _rng.normal(s) * 0.05)(D, F) * (D ** -0.5)),
            "w2": _w((lambda *s: _rng.normal(s) * 0.05)(F, D) * (F ** -0.5)),
        }
    _B_in = _B_setup()

    return {
        "A_x": _A_in["x"],
        "A_wq": _A_in["wq"],
        "A_wk": _A_in["wk"],
        "A_wv": _A_in["wv"],
        "A_wo": _A_in["wo"],
        "B_x": _B_in["x"],
        "B_w1": _B_in["w1"],
        "B_w2": _B_in["w2"],
    }

def reference(A_x, A_wq, A_wk, A_wv, A_wo, B_x, B_w1, B_w2):
    def _A_ref(x, wq, wk, wv, wo):
        B, S, D = x.shape
        H = 32
        Dh = D // H
        q = (lambda x, *d: x.transpose(*d))((x @ wq).reshape(B, S, H, Dh), 0, 2, 1, 3)
        k = x @ wk
        v = x @ wv
        scores = jnp.einsum("bhqd,bkd->bhqk", q, k) * (Dh ** -0.5)
        p = _softmax(scores, axis=-1)
        o = jnp.einsum("bhqk,bkd->bhqd", p, v)
        return (lambda x, *d: x.transpose(*d))(o, 0, 2, 1, 3).reshape(B, S, H * Dh) @ wo

    def _B_ref(x, w1, w2):
        h = jnp.einsum("bsd,df->bsf", x, w1)
        h = _silu(h)
        out = jnp.einsum("bsf,fd->bsd", h, w2)
        return out

    x = A_x
    xn = _layernorm(x, axis=-1)
    return x + _A_ref(xn, A_wq, A_wk, A_wv, A_wo) + _B_ref(xn, B_w1, B_w2)
```

```python
import jax
import jax.numpy as jnp
from jax import lax
import jax.experimental.pallas as pl
import jax.experimental.pallas.tpu as pltpu

S, D, H, DH, F = 2048, 512, 32, 16, 1792
TQ = 512
NQ = S // TQ
HPI = 16
NIT = H // HPI
FR = TQ // NIT
RC = 256
NRC = S // RC
KC = 256
NKC = S // KC
LAG = 1
F_SPLIT = 1280
LOG2E = 1.4426950408889634
EPS = 1e-5
QMAX = 3967.0
TINY = 1e-30
L_LO = 2.0 ** -60
L_HI = 2.0 ** 100
MAGIC = 12582912.0
MAGIC_BITS = 0x4B400000
X_PIECES = ((0, 256), (256, 768), (1024, 1024))


def _nt(a, b):
    return lax.dot_general(a, b, (((1,), (1,)), ((), ())), preferred_element_type=jnp.float32)


def _tn(a, b):
    return lax.dot_general(a, b, (((0,), (0,)), ((), ())), preferred_element_type=jnp.float32)


def _limbs(z):
    t = lax.bitcast_convert_type(z + MAGIC, jnp.int32) - (MAGIC_BITS - 128)
    hi = t >> 8
    low = t & 255
    return hi, low - 128, (low - 120) >> 4


def _kernel(x_hbm, wq_hbm, wkT_hbm, wvT_hbm, wo_hbm, w1_hbm, w2_hbm, o_ref,
            x_v, wq_v, wo_v, w1_v, w2_v, sem,
            wT_ref, xn_ref, qT_ref, kT_ref, ks_ref, k8_ref, vT_ref, vs_ref, q8_ref, c_ref,
            oT_ref, acc_ref, s_ref):
    i = pl.program_id(0)

    def quant_q(blk):
        cols = pl.ds(blk * TQ if isinstance(blk, int) else pl.multiple_of(blk * TQ, TQ), TQ)
        for h in range(H):
            q = qT_ref[h * DH:(h + 1) * DH, cols] * ks_ref[...]
            qmax = jnp.maximum(jnp.max(jnp.abs(q), axis=0, keepdims=True), TINY)
            hi, lo, lo16 = _limbs(q * (QMAX / qmax))
            h8 = hi << 3
            ql = jnp.concatenate([h8, h8, h8, h8, hi, lo, lo16, jnp.zeros_like(hi)], axis=0)
            q8_ref[h] = ql.astype(jnp.int8)
            c_ref[h] = qmax * (256.0 / (QMAX * QMAX))

    @pl.when(i == 0)
    def _prologue():
        xcp = [pltpu.make_async_copy(x_hbm.at[pl.ds(r0, n)], x_v.at[pl.ds(r0, n)], sem.at[j])
               for j, (r0, n) in enumerate(X_PIECES)]
        wcp = [pltpu.make_async_copy(src, dst, sem.at[3 + j]) for j, (src, dst) in enumerate(
            [(wq_hbm, wq_v), (wkT_hbm, wT_ref.at[pl.ds(D, DH)]), (wvT_hbm, wT_ref.at[pl.ds(D + DH, DH)]),
             (w1_hbm, w1_v), (w2_hbm, w2_v), (wo_hbm, wo_v)])]
        xcp[0].start()
        wcp[0].start()
        wcp[1].start()
        wcp[2].start()

        def ln(c):
            rows = pl.ds(c * RC, RC)
            x = x_v[rows, :].astype(jnp.float32)
            mu = jnp.mean(x, axis=-1, keepdims=True)
            xc = x - mu
            var = jnp.mean(xc * xc, axis=-1, keepdims=True)
            xn_ref[rows, :] = (xc * lax.rsqrt(var + EPS)).astype(jnp.bfloat16)

        def proj(c, lo, hi):
            rows = pl.ds(c * RC, RC)
            r = _nt(wT_ref[lo:hi, :], xn_ref[rows, :])
            if lo < D:
                qT_ref[:, rows] = r[:D]
            if hi > D:
                kT_ref[:, rows] = r[D - lo:D - lo + DH]
                vT_ref[:, rows] = r[D - lo + DH:]

        xcp[0].wait()
        xcp[1].start()
        ln(0)
        wcp[0].wait()
        wcp[1].wait()
        wcp[2].wait()
        xcp[2].start()
        wT_ref[0:D, :] = wq_v[...].T
        xcp[1].wait()
        wcp[3].start()
        wcp[4].start()
        wcp[5].start()
        ln(1)
        for c in range(NRC // 2):
            if (2 * c + 2) * RC == X_PIECES[2][0]:
                xcp[2].wait()
            for cc in (2 * c + 2, 2 * c + 3):
                if cc < NRC:
                    ln(cc)
            proj(c, 0, D + 2 * DH)
        for c in range(NRC // 2, NRC):
            proj(c, D, D + 2 * DH)

        kmax = jnp.maximum(jnp.max(jnp.abs(kT_ref[...]), axis=1, keepdims=True), TINY)
        ks_ref[...] = jnp.broadcast_to(kmax * (LOG2E * DH ** -0.5), (DH, TQ))
        kinv = QMAX / kmax
        vmax = jnp.maximum(jnp.max(jnp.abs(vT_ref[...]), axis=1, keepdims=True), TINY)
        vs_ref[...] = jnp.broadcast_to(vmax, (DH, TQ))
        vT_ref[...] = vT_ref[...] * (1.0 / vmax)
        for c in range(NRC):
            rows = pl.ds(c * RC, RC)
            hi, lo, lo16 = _limbs(kT_ref[:, rows] * kinv)
            h8 = hi << 3
            kl = jnp.concatenate([h8, h8, h8, h8, lo, hi, lo16, jnp.zeros_like(hi)], axis=0)
            k8_ref[rows, :] = kl.T.astype(jnp.int8)
        quant_q(0)
        for c in range(NRC // 2, NRC):
            proj(c, 0, D)
        wcp[3].wait()
        wcp[4].wait()
        wcp[5].wait()

    row0 = pl.multiple_of(i * TQ, TQ)

    def store_o(h, acc, l):
        oT_ref[pl.ds(pl.multiple_of(h * DH, DH), DH), :] = (
            acc * vs_ref[...] * pl.reciprocal(l, approx=False)).astype(jnp.bfloat16)

    def body(t, bad):
        frows = pl.ds(pl.multiple_of(row0 + t * FR, FR), FR)
        hh = 0.5 * jnp.dot(xn_ref[frows, :], w1_v[...], preferred_element_type=jnp.float32)
        hs = (hh + hh * jnp.tanh(hh)).astype(jnp.bfloat16)
        ffn = x_v[frows, :].astype(jnp.float32)

        nitems = HPI * NKC
        ps = {}
        acc = l = None
        for n in range(nitems + LAG):
            if n < nitems:
                j, c = divmod(n, NKC)
                s = jnp.dot(k8_ref[pl.ds(c * KC, KC), :], q8_ref[HPI * t + j],
                            preferred_element_type=jnp.int32)
                ps[n] = jnp.exp2(s.astype(jnp.float32) * c_ref[HPI * t + j])
            if n == nitems + LAG - 1:
                ffn = jnp.dot(hs[:, :F_SPLIT], w2_v[0:F_SPLIT, :], preferred_element_type=jnp.float32) + ffn
            if n >= LAG:
                j, c = divmod(n - LAG, NKC)
                p = ps.pop(n - LAG)
                lc = jnp.sum(p.reshape(KC // 8, 8, TQ), axis=0)
                o = jnp.dot(vT_ref[:, pl.ds(c * KC, KC)], p, preferred_element_type=jnp.float32)
                acc = o if c == 0 else o + acc
                l = lc if c == 0 else l + lc
                if c == NKC - 1:
                    lt = jnp.sum(l, axis=0, keepdims=True)
                    ok = jnp.logical_and(lt >= L_LO, lt <= L_HI)
                    bad = jnp.where(ok, bad, 1.0)
                    store_o(HPI * t + j, acc, lt)
        ffn = jnp.dot(hs[:, F_SPLIT:], w2_v[F_SPLIT:, :], preferred_element_type=jnp.float32) + ffn
        acc_ref[pl.ds(pl.multiple_of(t * FR, FR), FR), :] = ffn
        return bad

    bad = lax.fori_loop(0, NIT, body, jnp.zeros((1, TQ), jnp.float32))

    @pl.when(jnp.max(bad) > 0.0)
    def _fallback():
        def fb(h, carry):
            q8 = q8_ref[h]
            m = None
            for c in range(NKC):
                r = pl.ds(c * KC, KC)
                s = jnp.dot(k8_ref[r, :], q8, preferred_element_type=jnp.int32).astype(jnp.float32)
                s_ref[r, :] = s
                cm = jnp.max(s.reshape(KC // 8, 8, TQ), axis=0)
                m = cm if m is None else jnp.maximum(m, cm)
            m = jnp.max(m, axis=0, keepdims=True)
            acc = l = None
            for c in range(NKC):
                r = pl.ds(c * KC, KC)
                p = jnp.exp2((s_ref[r, :] - m) * c_ref[h])
                lc = jnp.sum(p.reshape(KC // 8, 8, TQ), axis=0)
                o = jnp.dot(vT_ref[:, r], p, preferred_element_type=jnp.float32)
                acc = o if c == 0 else o + acc
                l = lc if c == 0 else l + lc
            store_o(h, acc, jnp.sum(l, axis=0, keepdims=True))
            return carry

        lax.fori_loop(0, H, fb, 0)

    quant_q(jnp.minimum(i + 1, NQ - 1))
    o_ref[...] = (_tn(oT_ref[...], wo_v[...]) + acc_ref[...]).astype(o_ref.dtype)


@jax.jit
def pallas_parallel_sum__grouped_kv_mqa__dense_activation_silu__prompt_kernel(
    A_x, A_wq, A_wk, A_wv, A_wo, B_x, B_w1, B_w2):
    x = A_x.reshape(S, D)
    bf = jnp.bfloat16
    out = pl.pallas_call(
        _kernel,
        grid=(NQ,),
        in_specs=[pl.BlockSpec(memory_space=pl.ANY)] * 7,
        out_specs=pl.BlockSpec((TQ, D), lambda i: (i, 0)),
        out_shape=jax.ShapeDtypeStruct((S, D), bf),
        scratch_shapes=[
            pltpu.VMEM((S, D), bf),
            pltpu.VMEM((D, D), bf),
            pltpu.VMEM((D, D), bf),
            pltpu.VMEM((D, F), bf),
            pltpu.VMEM((F, D), bf),
            pltpu.SemaphoreType.DMA((9,)),
            pltpu.VMEM((D + 2 * DH, D), bf),
            pltpu.VMEM((S, D), bf),
            pltpu.VMEM((D, S), jnp.float32),
            pltpu.VMEM((DH, S), jnp.float32),
            pltpu.VMEM((DH, TQ), jnp.float32),
            pltpu.VMEM((S, 128), jnp.int8),
            pltpu.VMEM((DH, S), jnp.float32),
            pltpu.VMEM((DH, TQ), jnp.float32),
            pltpu.VMEM((H, 128, TQ), jnp.int8),
            pltpu.VMEM((H, 1, TQ), jnp.float32),
            pltpu.VMEM((D, TQ), bf),
            pltpu.VMEM((TQ, D), jnp.float32),
            pltpu.VMEM((S, TQ), jnp.float32),
        ],
        compiler_params=pltpu.CompilerParams(
            dimension_semantics=("arbitrary",), vmem_limit_bytes=100 * 1024 * 1024),
    )(x, A_wq, A_wk.T, A_wv.T, A_wo, B_w1, B_w2)
    return out.reshape(1, S, D)
```

```python
import jax
import jax.numpy as jnp
from jax import lax
import jax.experimental.pallas as pl
import jax.experimental.pallas.tpu as pltpu

S, D, H, DH, F = 2048, 512, 32, 16, 1792
TQ = 256
NQ = S // TQ
NC = 512
HG = NC // TQ
NG = H // HG
KC = 256
NKC = S // KC
F_SPLIT = 512
LOG2E = 1.4426950408889634
EPS = 1e-5
QMAX = 3967.0
TINY = 1e-30
L_LO = 2.0 ** -60
L_HI = 2.0 ** 100
MAGIC = 12582912.0
MAGIC_BITS = 0x4B400000
DMA_ORDER = ("x0", "wk", "wv", "x1", "x2", "x3", "x4", "x5", "wq0", "x6", "x7", "wq1",
             "w1", "w2", "wo")


def _dot(a, b, out=jnp.float32):
    return jnp.dot(a, b, preferred_element_type=out)


def _dot_nt(a, b):
    return lax.dot_general(a, b, (((1,), (1,)), ((), ())), preferred_element_type=jnp.float32)


def _dot_tn(a, b):
    return lax.dot_general(a, b, (((0,), (0,)), ((), ())), preferred_element_type=jnp.float32)


def _limbs(z):
    t = lax.bitcast_convert_type(z + MAGIC, jnp.int32) - (MAGIC_BITS - 128)
    low = t & 255
    return t >> 8, low - 128, (low - 120) >> 4


def _recip(x):
    r = pl.reciprocal(x, approx=True)
    return r * (2.0 - x * r)


def _kernel(x_hbm, wq_hbm, wkT_hbm, wvT_hbm, wo_hbm, w1_hbm, w2_hbm, o_ref,
            x_v, wq_v, wo_v, w1_v, w2_v, sem,
            wT_ref, xn_ref, kT_ref, ks_ref, k8_ref, vT_ref, vs_ref, q8_ref, c_ref,
            oT_ref, res_ref, s_ref):
    i = pl.program_id(0)

    @pl.when(i == 0)
    def _prologue():
        half = D // 2
        pairs = {
            "wk": (wkT_hbm, wT_ref.at[pl.ds(D, DH)]),
            "wv": (wvT_hbm, wT_ref.at[pl.ds(D + DH, DH)]),
            "w1": (w1_hbm, w1_v), "w2": (w2_hbm, w2_v), "wo": (wo_hbm, wo_v),
        }
        for j in range(2):
            pairs["wq%d" % j] = (wq_hbm.at[:, pl.ds(j * half, half)], wq_v.at[:, pl.ds(j * half, half)])
        for c in range(NQ):
            pairs["x%d" % c] = (x_hbm.at[pl.ds(c * TQ, TQ)], x_v.at[pl.ds(c * TQ, TQ)])
        cps = {n: pltpu.make_async_copy(*pairs[n], sem.at[j]) for j, n in enumerate(DMA_ORDER)}
        for n in DMA_ORDER:
            cps[n].start()

        def wait(*names):
            for n in names:
                cps[n].wait()

        def layernorm(c):
            rows = pl.ds(c * TQ, TQ)
            x = x_v[rows, :].astype(jnp.float32)
            xc = x - jnp.mean(x, axis=-1, keepdims=True)
            var = jnp.mean(xc * xc, axis=-1, keepdims=True)
            xn_ref[rows, :] = (xc * lax.rsqrt(var + EPS)).astype(jnp.bfloat16)

        def proj_kv(c):
            rows = pl.ds(c * TQ, TQ)
            r = _dot_nt(wT_ref[D:, :], xn_ref[rows, :])
            kT_ref[:, rows] = r[:DH]
            vT_ref[:, rows] = r[DH:]

        def transpose_wq(j):
            wT_ref[j * half:(j + 1) * half, :] = wq_v[:, j * half:(j + 1) * half].T

        def prep_kv():
            kmax = jnp.maximum(jnp.max(jnp.abs(kT_ref[...]), axis=1, keepdims=True), TINY)
            ks_ref[...] = jnp.broadcast_to(kmax * (LOG2E * DH ** -0.5), (DH, TQ))
            kinv = QMAX / kmax
            vmax = jnp.maximum(jnp.max(jnp.abs(vT_ref[...]), axis=1, keepdims=True), TINY)
            vs_ref[...] = jnp.broadcast_to(vmax, (DH, NC))
            vT_ref[...] = vT_ref[...] * (1.0 / vmax)
            for c in range(NQ):
                rows = pl.ds(c * TQ, TQ)
                hi, lo, lo16 = _limbs(kT_ref[:, rows] * kinv)
                h8 = hi << 3
                kl = jnp.concatenate([h8, h8, h8, h8, lo, hi, lo16, jnp.zeros_like(hi)], axis=0)
                k8_ref[rows, :] = kl.T.astype(jnp.int8)

        def proj_q(c):
            qT = _dot_nt(wT_ref[0:D, :], xn_ref[pl.ds(c * TQ, TQ), :])
            for h in range(H):
                g, j = divmod(h, HG)
                q = qT[h * DH:(h + 1) * DH] * ks_ref[...]
                qmax = jnp.maximum(jnp.max(jnp.abs(q), axis=0, keepdims=True), TINY)
                hi, lo, lo16 = _limbs(q * (QMAX * _recip(qmax)))
                h8 = hi << 3
                ql = jnp.concatenate([h8, h8, h8, h8, hi, lo, lo16, jnp.zeros_like(hi)], axis=0)
                q8_ref[c * NG + g, :, j * TQ:(j + 1) * TQ] = ql.astype(jnp.int8)
                c_ref[c * NG + g, :, j * TQ:(j + 1) * TQ] = qmax * (256.0 / (QMAX * QMAX))

        wait("x0")
        layernorm(0)
        wait("wk", "wv")
        for c in range(1, 6):
            wait("x%d" % c)
            layernorm(c)
            proj_kv(c - 1)
        wait("wq0")
        transpose_wq(0)
        proj_kv(5)
        wait("x6")
        layernorm(6)
        wait("x7")
        layernorm(7)
        proj_kv(6)
        proj_kv(7)
        wait("wq1")
        transpose_wq(1)
        prep_kv()
        for c in range(NQ):
            proj_q(c)
        wait("w1", "w2", "wo")

    rows = pl.ds(pl.multiple_of(i * TQ, TQ), TQ)

    def scores(g, c):
        s = _dot(k8_ref[pl.ds(c * KC, KC), :], q8_ref[i * NG + g], jnp.int32)
        return s.astype(jnp.float32)

    def accumulate(c, p, acc, l):
        lc = jnp.sum(p.reshape(KC // 8, 8, NC), axis=0)
        o = _dot(vT_ref[:, pl.ds(c * KC, KC)], p)
        return (o, lc) if c == 0 else (o + acc, l + lc)

    def finish(acc, lt):
        return (acc * vs_ref[...] * pl.reciprocal(lt, approx=False)).astype(jnp.bfloat16)

    hh = 0.5 * _dot(xn_ref[rows, :], w1_v[...])
    hs = (hh + hh * jnp.tanh(hh)).astype(jnp.bfloat16)
    res = x_v[rows, :].astype(jnp.float32)

    n_chunks = NG * NKC
    p_prev = acc = l = None
    bad = jnp.zeros((1, NC), jnp.float32)
    for n in range(n_chunks + 1):
        p_new = None
        if n < n_chunks:
            g, c = divmod(n, NKC)
            p_new = jnp.exp2(scores(g, c) * c_ref[i * NG + g])
        else:
            res = _dot(hs[:, :F_SPLIT], w2_v[0:F_SPLIT, :]) + res
        if n > 0:
            g, c = divmod(n - 1, NKC)
            acc, l = accumulate(c, p_prev, acc, l)
            if c == NKC - 1:
                lt = jnp.sum(l, axis=0, keepdims=True)
                bad = jnp.where(jnp.logical_and(lt >= L_LO, lt <= L_HI), bad, 1.0)
                og = finish(acc, lt)
                for j in range(HG):
                    h = g * HG + j
                    oT_ref[h * DH:(h + 1) * DH, :] = og[:, j * TQ:(j + 1) * TQ]
        p_prev = p_new
    res = _dot(hs[:, F_SPLIT:], w2_v[F_SPLIT:, :]) + res
    res_ref[...] = res
    unsafe = jnp.max(bad) > 0.0
    o_ref[...] = (_dot_tn(oT_ref[...], wo_v[...]) + res).astype(o_ref.dtype)

    @pl.when(unsafe)
    def _fallback():
        def item(g, carry):
            m = None
            for c in range(NKC):
                s = scores(g, c)
                s_ref[pl.ds(c * KC, KC), :] = s
                cm = jnp.max(s.reshape(KC // 8, 8, NC), axis=0)
                m = cm if m is None else jnp.maximum(m, cm)
            m = jnp.max(m, axis=0, keepdims=True)
            acc = l = None
            for c in range(NKC):
                p = jnp.exp2((s_ref[pl.ds(c * KC, KC), :] - m) * c_ref[i * NG + g])
                acc, l = accumulate(c, p, acc, l)
            og = finish(acc, jnp.sum(l, axis=0, keepdims=True))
            for j in range(HG):
                oT_ref[pl.ds(pl.multiple_of((g * HG + j) * DH, DH), DH), :] = og[:, j * TQ:(j + 1) * TQ]
            return carry

        lax.fori_loop(0, NG, item, 0)
        o_ref[...] = (_dot_tn(oT_ref[...], wo_v[...]) + res_ref[...]).astype(o_ref.dtype)


@jax.jit
def pallas_parallel_sum__grouped_kv_mqa__dense_activation_silu__prompt_kernel(
    A_x: jax.Array,
    A_wq: jax.Array,
    A_wk: jax.Array,
    A_wv: jax.Array,
    A_wo: jax.Array,
    B_x: jax.Array,
    B_w1: jax.Array,
    B_w2: jax.Array,
):
    del B_x
    bf, f32 = jnp.bfloat16, jnp.float32
    out = pl.pallas_call(
        _kernel,
        grid=(NQ,),
        in_specs=[pl.BlockSpec(memory_space=pl.ANY)] * 7,
        out_specs=pl.BlockSpec((TQ, D), lambda i: (i, 0)),
        out_shape=jax.ShapeDtypeStruct((S, D), bf),
        scratch_shapes=[
            pltpu.VMEM((S, D), bf),
            pltpu.VMEM((D, D), bf),
            pltpu.VMEM((D, D), bf),
            pltpu.VMEM((D, F), bf),
            pltpu.VMEM((F, D), bf),
            pltpu.SemaphoreType.DMA((len(DMA_ORDER),)),
            pltpu.VMEM((D + 2 * DH, D), bf),
            pltpu.VMEM((S, D), bf),
            pltpu.VMEM((DH, S), f32),
            pltpu.VMEM((DH, TQ), f32),
            pltpu.VMEM((S, 128), jnp.int8),
            pltpu.VMEM((DH, S), f32),
            pltpu.VMEM((DH, NC), f32),
            pltpu.VMEM((NQ * NG, 128, NC), jnp.int8),
            pltpu.VMEM((NQ * NG, 1, NC), f32),
            pltpu.VMEM((D, TQ), bf),
            pltpu.VMEM((TQ, D), f32),
            pltpu.VMEM((S, NC), f32),
        ],
        compiler_params=pltpu.CompilerParams(
            dimension_semantics=("arbitrary",), vmem_limit_bytes=64 * 1024 * 1024),
    )(A_x.reshape(S, D), A_wq, A_wk.T, A_wv.T, A_wo, B_w1, B_w2)
    return out.reshape(1, S, D)
```

```python
import jax
import jax.numpy as jnp
from jax import lax
import jax.experimental.pallas as pl
import jax.experimental.pallas.tpu as pltpu

S, D, H, DH, F = 2048, 512, 32, 16, 1792
TQ = 256
NQ = S // TQ
NC = 512
HG = NC // TQ
NG = H // HG
KC = 256
NKC = S // KC
FA = 384
LOG2E = 1.4426950408889634
EPS = 1e-5
QMAX = 3967.0
TINY = 1e-30
L_LO = 2.0 ** -60
L_HI = 2.0 ** 100
MAGIC = 12582912.0
MAGIC_BITS = 0x4B400000
DMA_ORDER = ("x0", "w1a", "wk", "wv", "x1", "x2", "x3", "x4", "x5", "wq0", "x6", "x7", "wq1",
             "w1b", "w2", "wo")


def _dot(a, b, out=jnp.float32):
    return jnp.dot(a, b, preferred_element_type=out)


def _dot_nt(a, b):
    return lax.dot_general(a, b, (((1,), (1,)), ((), ())), preferred_element_type=jnp.float32)


def _dot_tn(a, b):
    return lax.dot_general(a, b, (((0,), (0,)), ((), ())), preferred_element_type=jnp.float32)


def _limbs(z):
    t = lax.bitcast_convert_type(z + MAGIC, jnp.int32) - (MAGIC_BITS - 128)
    low = t & 255
    return t >> 8, low - 128, (low - 120) >> 4


def _recip(x):
    r = pl.reciprocal(x, approx=True)
    return r * (2.0 - x * r)


def _silu(h):
    hh = 0.5 * h
    return (hh + hh * jnp.tanh(hh)).astype(jnp.bfloat16)


def _kernel(x_hbm, wq_hbm, wkT_hbm, wvT_hbm, wo_hbm, w1_hbm, w2_hbm, o_ref,
            x_v, wq_v, wo_v, w1_v, w2_v, sem,
            wT_ref, xn_ref, kT_ref, ks_ref, k8_ref, vT_ref, vs_ref, q8_ref, c_ref,
            oT_ref, res_ref, s_ref, ha_ref):
    i = pl.program_id(0)

    @pl.when(i == 0)
    def _prologue():
        half = D // 2
        pairs = {
            "wk": (wkT_hbm, wT_ref.at[pl.ds(D, DH)]),
            "wv": (wvT_hbm, wT_ref.at[pl.ds(D + DH, DH)]),
            "w1a": (w1_hbm.at[:, pl.ds(0, FA)], w1_v.at[:, pl.ds(0, FA)]),
            "w1b": (w1_hbm.at[:, pl.ds(FA, F - FA)], w1_v.at[:, pl.ds(FA, F - FA)]),
            "w2": (w2_hbm, w2_v), "wo": (wo_hbm, wo_v),
        }
        for j in range(2):
            pairs["wq%d" % j] = (wq_hbm.at[:, pl.ds(j * half, half)], wq_v.at[:, pl.ds(j * half, half)])
        for c in range(NQ):
            pairs["x%d" % c] = (x_hbm.at[pl.ds(c * TQ, TQ)], x_v.at[pl.ds(c * TQ, TQ)])
        cps = {n: pltpu.make_async_copy(*pairs[n], sem.at[j]) for j, n in enumerate(DMA_ORDER)}
        for n in DMA_ORDER:
            cps[n].start()

        def wait(*names):
            for n in names:
                cps[n].wait()

        def layernorm(c):
            rows = pl.ds(c * TQ, TQ)
            x = x_v[rows, :].astype(jnp.float32)
            xc = x - jnp.mean(x, axis=-1, keepdims=True)
            var = jnp.mean(xc * xc, axis=-1, keepdims=True)
            xn_ref[rows, :] = (xc * lax.rsqrt(var + EPS)).astype(jnp.bfloat16)

        def proj_kv(c):
            rows = pl.ds(c * TQ, TQ)
            r = _dot_nt(wT_ref[D:, :], xn_ref[rows, :])
            kT_ref[:, rows] = r[:DH]
            vT_ref[:, rows] = r[DH:]

        def up_a(c):
            rows = pl.ds(c * TQ, TQ)
            ha_ref[rows, :] = _silu(_dot(xn_ref[rows, :], w1_v[:, 0:FA]))

        def transpose_wq(j):
            wT_ref[j * half:(j + 1) * half, :] = wq_v[:, j * half:(j + 1) * half].T

        def prep_kv():
            kmax = jnp.maximum(jnp.max(jnp.abs(kT_ref[...]), axis=1, keepdims=True), TINY)
            ks_ref[...] = jnp.broadcast_to(kmax * (LOG2E * DH ** -0.5), (DH, TQ))
            kinv = QMAX / kmax
            vmax = jnp.maximum(jnp.max(jnp.abs(vT_ref[...]), axis=1, keepdims=True), TINY)
            vs_ref[...] = jnp.broadcast_to(vmax, (DH, NC))
            vT_ref[...] = vT_ref[...] * (1.0 / vmax)
            for c in range(NQ):
                rows = pl.ds(c * TQ, TQ)
                hi, lo, lo16 = _limbs(kT_ref[:, rows] * kinv)
                h8 = hi << 3
                kl = jnp.concatenate([h8, h8, h8, h8, lo, hi, lo16, jnp.zeros_like(hi)], axis=0)
                k8_ref[rows, :] = kl.T.astype(jnp.int8)

        def proj_q(c):
            qT = _dot_nt(wT_ref[0:D, :], xn_ref[pl.ds(c * TQ, TQ), :])
            for h in range(H):
                g, j = divmod(h, HG)
                q = qT[h * DH:(h + 1) * DH] * ks_ref[...]
                qmax = jnp.maximum(jnp.max(jnp.abs(q), axis=0, keepdims=True), TINY)
                hi, lo, lo16 = _limbs(q * (QMAX * _recip(qmax)))
                h8 = hi << 3
                ql = jnp.concatenate([h8, h8, h8, h8, hi, lo, lo16, jnp.zeros_like(hi)], axis=0)
                q8_ref[c * NG + g, :, j * TQ:(j + 1) * TQ] = ql.astype(jnp.int8)
                c_ref[c * NG + g, :, j * TQ:(j + 1) * TQ] = qmax * (256.0 / (QMAX * QMAX))

        wait("x0")
        layernorm(0)
        wait("w1a", "wk", "wv", "x1")
        layernorm(1)
        up_a(0)
        proj_kv(0)
        wait("x2", "x3")
        up_a(1)
        proj_kv(1)
        layernorm(2)
        up_a(2)
        proj_kv(2)
        layernorm(3)
        wait("x4", "x5", "wq0")
        up_a(3)
        proj_kv(3)
        layernorm(4)
        up_a(4)
        proj_kv(4)
        layernorm(5)
        transpose_wq(0)
        wait("x6", "x7", "wq1")
        up_a(5)
        proj_kv(5)
        layernorm(6)
        up_a(6)
        proj_kv(6)
        layernorm(7)
        proj_kv(7)
        up_a(7)
        transpose_wq(1)
        prep_kv()
        for c in range(NQ):
            proj_q(c)
        wait("w1b", "w2", "wo")

    rows = pl.ds(pl.multiple_of(i * TQ, TQ), TQ)

    def scores(g, c):
        s = _dot(k8_ref[pl.ds(c * KC, KC), :], q8_ref[i * NG + g], jnp.int32)
        return s.astype(jnp.float32)

    def accumulate(c, p, acc, l):
        lc = jnp.sum(p.reshape(KC // 8, 8, NC), axis=0)
        o = _dot(vT_ref[:, pl.ds(c * KC, KC)], p)
        return (o, lc) if c == 0 else (o + acc, l + lc)

    def finish(acc, lt):
        return (acc * vs_ref[...] * pl.reciprocal(lt, approx=False)).astype(jnp.bfloat16)

    hs = _silu(_dot(xn_ref[rows, :], w1_v[:, FA:]))
    res = x_v[rows, :].astype(jnp.float32)

    n_chunks = NG * NKC
    p_prev = acc = l = None
    bad = jnp.zeros((1, NC), jnp.float32)
    for n in range(n_chunks + 1):
        p_new = None
        if n < n_chunks:
            g, c = divmod(n, NKC)
            p_new = jnp.exp2(scores(g, c) * c_ref[i * NG + g])
        else:
            res = _dot(ha_ref[rows, :], w2_v[0:FA, :]) + res
        if n > 0:
            g, c = divmod(n - 1, NKC)
            acc, l = accumulate(c, p_prev, acc, l)
            if c == NKC - 1:
                lt = jnp.sum(l, axis=0, keepdims=True)
                bad = jnp.where(jnp.logical_and(lt >= L_LO, lt <= L_HI), bad, 1.0)
                og = finish(acc, lt)
                for j in range(HG):
                    h = g * HG + j
                    oT_ref[h * DH:(h + 1) * DH, :] = og[:, j * TQ:(j + 1) * TQ]
        p_prev = p_new
    res = _dot(hs, w2_v[FA:, :]) + res
    res_ref[...] = res
    unsafe = jnp.max(bad) > 0.0
    o_ref[...] = (_dot_tn(oT_ref[...], wo_v[...]) + res).astype(o_ref.dtype)

    @pl.when(unsafe)
    def _fallback():
        def item(g, carry):
            m = None
            for c in range(NKC):
                s = scores(g, c)
                s_ref[pl.ds(c * KC, KC), :] = s
                cm = jnp.max(s.reshape(KC // 8, 8, NC), axis=0)
                m = cm if m is None else jnp.maximum(m, cm)
            m = jnp.max(m, axis=0, keepdims=True)
            acc = l = None
            for c in range(NKC):
                p = jnp.exp2((s_ref[pl.ds(c * KC, KC), :] - m) * c_ref[i * NG + g])
                acc, l = accumulate(c, p, acc, l)
            og = finish(acc, jnp.sum(l, axis=0, keepdims=True))
            for j in range(HG):
                oT_ref[pl.ds(pl.multiple_of((g * HG + j) * DH, DH), DH), :] = og[:, j * TQ:(j + 1) * TQ]
            return carry

        lax.fori_loop(0, NG, item, 0)
        o_ref[...] = (_dot_tn(oT_ref[...], wo_v[...]) + res_ref[...]).astype(o_ref.dtype)


@jax.jit
def pallas_parallel_sum__grouped_kv_mqa__dense_activation_silu__prompt_kernel(
    A_x: jax.Array,
    A_wq: jax.Array,
    A_wk: jax.Array,
    A_wv: jax.Array,
    A_wo: jax.Array,
    B_x: jax.Array,
    B_w1: jax.Array,
    B_w2: jax.Array,
):
    del B_x
    bf, f32 = jnp.bfloat16, jnp.float32
    out = pl.pallas_call(
        _kernel,
        grid=(NQ,),
        in_specs=[pl.BlockSpec(memory_space=pl.ANY)] * 7,
        out_specs=pl.BlockSpec((TQ, D), lambda i: (i, 0)),
        out_shape=jax.ShapeDtypeStruct((S, D), bf),
        scratch_shapes=[
            pltpu.VMEM((S, D), bf),
            pltpu.VMEM((D, D), bf),
            pltpu.VMEM((D, D), bf),
            pltpu.VMEM((D, F), bf),
            pltpu.VMEM((F, D), bf),
            pltpu.SemaphoreType.DMA((len(DMA_ORDER),)),
            pltpu.VMEM((D + 2 * DH, D), bf),
            pltpu.VMEM((S, D), bf),
            pltpu.VMEM((DH, S), f32),
            pltpu.VMEM((DH, TQ), f32),
            pltpu.VMEM((S, 128), jnp.int8),
            pltpu.VMEM((DH, S), f32),
            pltpu.VMEM((DH, NC), f32),
            pltpu.VMEM((NQ * NG, 128, NC), jnp.int8),
            pltpu.VMEM((NQ * NG, 1, NC), f32),
            pltpu.VMEM((D, TQ), bf),
            pltpu.VMEM((TQ, D), f32),
            pltpu.VMEM((S, NC), f32),
            pltpu.VMEM((S, FA), bf),
        ],
        compiler_params=pltpu.CompilerParams(
            dimension_semantics=("arbitrary",), vmem_limit_bytes=64 * 1024 * 1024),
    )(A_x.reshape(S, D), A_wq, A_wk.T, A_wv.T, A_wo, B_w1, B_w2)
    return out.reshape(1, S, D)
```

```python
import jax
import jax.numpy as jnp
from jax import lax
import jax.experimental.pallas as pl
import jax.experimental.pallas.tpu as pltpu

S, D, H, DH, F = 2048, 512, 32, 16, 1792
TQ = 256
NQ = S // TQ
NC = 512
HG = NC // TQ
NG = H // HG
KC = 256
NKC = S // KC
FA = 512
FA1 = 256
LOG2E = 1.4426950408889634
EPS = 1e-5
QMAX = 3967.0
TINY = 1e-30
L_LO = 2.0 ** -60
L_HI = 2.0 ** 100
MAGIC = 12582912.0
MAGIC_BITS = 0x4B400000
DMA_ORDER = ("x0", "w1a", "x1", "w1b", "wk", "wv", "x2", "x3", "x4", "x5", "wq0", "x6", "x7", "wq1",
             "w1c", "w2", "wo")


def _dot(a, b, out=jnp.float32):
    return jnp.dot(a, b, preferred_element_type=out)


def _dot_nt(a, b):
    return lax.dot_general(a, b, (((1,), (1,)), ((), ())), preferred_element_type=jnp.float32)


def _dot_tn(a, b):
    return lax.dot_general(a, b, (((0,), (0,)), ((), ())), preferred_element_type=jnp.float32)


def _limbs(z):
    t = lax.bitcast_convert_type(z + MAGIC, jnp.int32) - (MAGIC_BITS - 128)
    low = t & 255
    return t >> 8, low - 128, (low - 120) >> 4


def _recip(x):
    r = pl.reciprocal(x, approx=True)
    return r * (2.0 - x * r)


def _silu(h):
    hh = 0.5 * h
    return (hh + hh * jnp.tanh(hh)).astype(jnp.bfloat16)


def _kernel(x_hbm, wq_hbm, wkT_hbm, wvT_hbm, wo_hbm, w1_hbm, w2_hbm, o_ref,
            x_v, wq_v, wo_v, w1_v, w2_v, sem,
            wT_ref, xn_ref, kT_ref, ks_ref, k8_ref, vT_ref, vs_ref, q8_ref, c_ref,
            oT_ref, res_ref, s_ref, ha_ref):
    i = pl.program_id(0)

    @pl.when(i == 0)
    def _prologue():
        half = D // 2
        pairs = {
            "wk": (wkT_hbm, wT_ref.at[pl.ds(D, DH)]),
            "wv": (wvT_hbm, wT_ref.at[pl.ds(D + DH, DH)]),
            "w1a": (w1_hbm.at[:, pl.ds(0, FA1)], w1_v.at[:, pl.ds(0, FA1)]),
            "w1b": (w1_hbm.at[:, pl.ds(FA1, FA - FA1)], w1_v.at[:, pl.ds(FA1, FA - FA1)]),
            "w1c": (w1_hbm.at[:, pl.ds(FA, F - FA)], w1_v.at[:, pl.ds(FA, F - FA)]),
            "w2": (w2_hbm, w2_v), "wo": (wo_hbm, wo_v),
        }
        for j in range(2):
            pairs["wq%d" % j] = (wq_hbm.at[:, pl.ds(j * half, half)], wq_v.at[:, pl.ds(j * half, half)])
        for c in range(NQ):
            pairs["x%d" % c] = (x_hbm.at[pl.ds(c * TQ, TQ)], x_v.at[pl.ds(c * TQ, TQ)])
        cps = {n: pltpu.make_async_copy(*pairs[n], sem.at[j]) for j, n in enumerate(DMA_ORDER)}
        for n in DMA_ORDER:
            cps[n].start()

        def wait(*names):
            for n in names:
                cps[n].wait()

        def layernorm(c):
            rows = pl.ds(c * TQ, TQ)
            x = x_v[rows, :].astype(jnp.float32)
            xc = x - jnp.mean(x, axis=-1, keepdims=True)
            var = jnp.mean(xc * xc, axis=-1, keepdims=True)
            xn_ref[rows, :] = (xc * lax.rsqrt(var + EPS)).astype(jnp.bfloat16)

        def proj_kv(c):
            rows = pl.ds(c * TQ, TQ)
            r = _dot_nt(wT_ref[D:, :], xn_ref[rows, :])
            kT_ref[:, rows] = r[:DH]
            vT_ref[:, rows] = r[DH:]

        def up_a(c, lo=0, hi=FA):
            rows = pl.ds(c * TQ, TQ)
            ha_ref[rows, lo:hi] = _silu(_dot(xn_ref[rows, :], w1_v[:, lo:hi]))

        def transpose_wq(j):
            wT_ref[j * half:(j + 1) * half, :] = wq_v[:, j * half:(j + 1) * half].T

        def prep_kv():
            kmax = jnp.maximum(jnp.max(jnp.abs(kT_ref[...]), axis=1, keepdims=True), TINY)
            ks_ref[...] = jnp.broadcast_to(kmax * (LOG2E * DH ** -0.5), (DH, TQ))
            kinv = QMAX / kmax
            vmax = jnp.maximum(jnp.max(jnp.abs(vT_ref[...]), axis=1, keepdims=True), TINY)
            vs_ref[...] = jnp.broadcast_to(vmax, (DH, NC))
            vT_ref[...] = vT_ref[...] * (1.0 / vmax)
            for c in range(NQ):
                rows = pl.ds(c * TQ, TQ)
                hi, lo, lo16 = _limbs(kT_ref[:, rows] * kinv)
                h8 = hi << 3
                kl = jnp.concatenate([h8, h8, h8, h8, lo, hi, lo16, jnp.zeros_like(hi)], axis=0)
                k8_ref[rows, :] = kl.T.astype(jnp.int8)

        def proj_q(c):
            qT = _dot_nt(wT_ref[0:D, :], xn_ref[pl.ds(c * TQ, TQ), :])
            for h in range(H):
                g, j = divmod(h, HG)
                q = qT[h * DH:(h + 1) * DH] * ks_ref[...]
                qmax = jnp.maximum(jnp.max(jnp.abs(q), axis=0, keepdims=True), TINY)
                hi, lo, lo16 = _limbs(q * (QMAX * _recip(qmax)))
                h8 = hi << 3
                ql = jnp.concatenate([h8, h8, h8, h8, hi, lo, lo16, jnp.zeros_like(hi)], axis=0)
                q8_ref[c * NG + g, :, j * TQ:(j + 1) * TQ] = ql.astype(jnp.int8)
                c_ref[c * NG + g, :, j * TQ:(j + 1) * TQ] = qmax * (256.0 / (QMAX * QMAX))

        wait("x0")
        layernorm(0)
        wait("w1a")
        up_a(0, 0, FA1)
        wait("x1", "w1b", "wk", "wv")
        up_a(0, FA1, FA)
        proj_kv(0)
        layernorm(1)
        up_a(1, 0, FA1)
        wait("x2", "x3")
        up_a(1, FA1, FA)
        proj_kv(1)
        layernorm(2)
        up_a(2)
        proj_kv(2)
        layernorm(3)
        wait("x4", "x5", "wq0")
        up_a(3)
        proj_kv(3)
        layernorm(4)
        up_a(4)
        proj_kv(4)
        layernorm(5)
        transpose_wq(0)
        wait("x6", "x7", "wq1")
        up_a(5)
        proj_kv(5)
        layernorm(6)
        up_a(6)
        proj_kv(6)
        layernorm(7)
        proj_kv(7)
        up_a(7)
        transpose_wq(1)
        prep_kv()
        for c in range(NQ):
            proj_q(c)
        wait("w1c", "w2", "wo")

    rows = pl.ds(pl.multiple_of(i * TQ, TQ), TQ)

    def scores(g, c):
        s = _dot(k8_ref[pl.ds(c * KC, KC), :], q8_ref[i * NG + g], jnp.int32)
        return s.astype(jnp.float32)

    def accumulate(c, p, acc, l):
        lc = jnp.sum(p.reshape(KC // 8, 8, NC), axis=0)
        o = _dot(vT_ref[:, pl.ds(c * KC, KC)], p)
        return (o, lc) if c == 0 else (o + acc, l + lc)

    def finish(acc, lt):
        return (acc * vs_ref[...] * pl.reciprocal(lt, approx=False)).astype(jnp.bfloat16)

    hs = _silu(_dot(xn_ref[rows, :], w1_v[:, FA:]))
    res = x_v[rows, :].astype(jnp.float32)

    n_chunks = NG * NKC
    p_prev = acc = l = None
    bad = jnp.zeros((1, NC), jnp.float32)
    for n in range(n_chunks + 1):
        p_new = None
        if n < n_chunks:
            g, c = divmod(n, NKC)
            p_new = jnp.exp2(scores(g, c) * c_ref[i * NG + g])
        else:
            res = _dot(ha_ref[rows, :], w2_v[0:FA, :]) + res
        if n > 0:
            g, c = divmod(n - 1, NKC)
            acc, l = accumulate(c, p_prev, acc, l)
            if c == NKC - 1:
                lt = jnp.sum(l, axis=0, keepdims=True)
                bad = jnp.where(jnp.logical_and(lt >= L_LO, lt <= L_HI), bad, 1.0)
                og = finish(acc, lt)
                for j in range(HG):
                    h = g * HG + j
                    oT_ref[h * DH:(h + 1) * DH, :] = og[:, j * TQ:(j + 1) * TQ]
        p_prev = p_new
    res = _dot(hs, w2_v[FA:, :]) + res
    res_ref[...] = res
    unsafe = jnp.max(bad) > 0.0
    o_ref[...] = (_dot_tn(oT_ref[...], wo_v[...]) + res).astype(o_ref.dtype)

    @pl.when(unsafe)
    def _fallback():
        def item(g, carry):
            m = None
            for c in range(NKC):
                s = scores(g, c)
                s_ref[pl.ds(c * KC, KC), :] = s
                cm = jnp.max(s.reshape(KC // 8, 8, NC), axis=0)
                m = cm if m is None else jnp.maximum(m, cm)
            m = jnp.max(m, axis=0, keepdims=True)
            acc = l = None
            for c in range(NKC):
                p = jnp.exp2((s_ref[pl.ds(c * KC, KC), :] - m) * c_ref[i * NG + g])
                acc, l = accumulate(c, p, acc, l)
            og = finish(acc, jnp.sum(l, axis=0, keepdims=True))
            for j in range(HG):
                oT_ref[pl.ds(pl.multiple_of((g * HG + j) * DH, DH), DH), :] = og[:, j * TQ:(j + 1) * TQ]
            return carry

        lax.fori_loop(0, NG, item, 0)
        o_ref[...] = (_dot_tn(oT_ref[...], wo_v[...]) + res_ref[...]).astype(o_ref.dtype)


@jax.jit
def pallas_parallel_sum__grouped_kv_mqa__dense_activation_silu__prompt_kernel(
    A_x: jax.Array,
    A_wq: jax.Array,
    A_wk: jax.Array,
    A_wv: jax.Array,
    A_wo: jax.Array,
    B_x: jax.Array,
    B_w1: jax.Array,
    B_w2: jax.Array,
):
    del B_x
    bf, f32 = jnp.bfloat16, jnp.float32
    out = pl.pallas_call(
        _kernel,
        grid=(NQ,),
        in_specs=[pl.BlockSpec(memory_space=pl.ANY)] * 7,
        out_specs=pl.BlockSpec((TQ, D), lambda i: (i, 0)),
        out_shape=jax.ShapeDtypeStruct((S, D), bf),
        scratch_shapes=[
            pltpu.VMEM((S, D), bf),
            pltpu.VMEM((D, D), bf),
            pltpu.VMEM((D, D), bf),
            pltpu.VMEM((D, F), bf),
            pltpu.VMEM((F, D), bf),
            pltpu.SemaphoreType.DMA((len(DMA_ORDER),)),
            pltpu.VMEM((D + 2 * DH, D), bf),
            pltpu.VMEM((S, D), bf),
            pltpu.VMEM((DH, S), f32),
            pltpu.VMEM((DH, TQ), f32),
            pltpu.VMEM((S, 128), jnp.int8),
            pltpu.VMEM((DH, S), f32),
            pltpu.VMEM((DH, NC), f32),
            pltpu.VMEM((NQ * NG, 128, NC), jnp.int8),
            pltpu.VMEM((NQ * NG, 1, NC), f32),
            pltpu.VMEM((D, TQ), bf),
            pltpu.VMEM((TQ, D), f32),
            pltpu.VMEM((S, NC), f32),
            pltpu.VMEM((S, FA), bf),
        ],
        compiler_params=pltpu.CompilerParams(
            dimension_semantics=("arbitrary",), vmem_limit_bytes=64 * 1024 * 1024),
    )(A_x.reshape(S, D), A_wq, A_wk.T, A_wv.T, A_wo, B_w1, B_w2)
    return out.reshape(1, S, D)
```
